```python
import jax
import jax.numpy as jnp

def _softmax(x, axis=-1):
    return jax.nn.softmax(x, axis=axis)
def _gelu(x):
    return jax.nn.gelu(x, approximate=True)
def _silu(x):
    return jax.nn.silu(x)
def _sigmoid(x):
    return jax.nn.sigmoid(x)
def _layernorm(x, axis=-1, eps=1e-5):
    m = jnp.mean(x, axis=axis, keepdims=True)
    v = jnp.var(x, axis=axis, keepdims=True)
    return (x - m) / jnp.sqrt(v + eps)
def _scatter_add(tgt, idx, src, axis=0):
    return tgt.at[idx].add(src)
def _segment_sum(src, seg, n):
    return jax.ops.segment_sum(src, seg, n)
class _Rng:
    def __init__(self, key):
        self._k = key
    def _next(self):
        self._k, sub = jax.random.split(self._k)
        return sub
    def normal(self, shape):
        return jax.random.normal(self._next(), shape, dtype=jnp.bfloat16)
    def randint(self, lo, hi, shape):
        return jax.random.randint(self._next(), shape, lo, hi, dtype=jnp.int32)
    def uniform(self, shape, lo=0.0, hi=1.0):
        return jax.random.uniform(self._next(), shape, jnp.bfloat16, lo, hi)
    def permutation(self, n):
        return jax.random.permutation(self._next(), n)


kernel_name = 'parallel_sum__gqa_block_cached__moe_arch_mod__decode'

def setup_inputs():
    _rng = _Rng(jax.random.key(int.from_bytes(__import__("os").urandom(4), "little")))
    _w = (lambda a: (lambda t: t.astype(jnp.bfloat16) if jnp.issubdtype(t.dtype, jnp.floating) else t)(jnp.asarray(a)))
    def _A_setup():
        B, Sq, D = 1, 1, 448
        Hq, Hkv, Sk, Dh = 16, 8, 65536, 256
        assert Hq % Hkv == 0, (Hq, Hkv)
        return {
            "x": _w((lambda *s: _rng.normal(s) * 0.05)(B, Sq, D)),
            "k_cache": _w((lambda *s: _rng.normal(s) * 0.05)(B, Hkv, Sk, Dh)),
            "v_cache": _w((lambda *s: _rng.normal(s) * 0.05)(B, Hkv, Sk, Dh)),
            "wq": _w((lambda *s: _rng.normal(s) * 0.05)(D, Hq * Dh) * (D ** -0.5)),
            "wo": _w((lambda *s: _rng.normal(s) * 0.05)(Hq * Dh, D) * ((Hq * Dh) ** -0.5)),
        }
    _A_in = _A_setup()

    def _B_setup():
        B, S, D, F, C = 1, 1, 448, 1792, 1
        return {
            "x": _w((lambda *s: _rng.normal(s) * 0.05)(B, S, D)),
            "w_r": _w((lambda *s: _rng.normal(s) * 0.05)(D)),
            "w_gate": _w((lambda *s: _rng.normal(s) * 0.05)(D, F)),
            "w_up": _w((lambda *s: _rng.normal(s) * 0.05)(D, F)),
            "w_down": _w((lambda *s: _rng.normal(s) * 0.05)(F, D)),
        }
    _B_in = _B_setup()

    return {
        "A_x": _A_in["x"],
        "A_k_cache": _A_in["k_cache"],
        "A_v_cache": _A_in["v_cache"],
        "A_wq": _A_in["wq"],
        "A_wo": _A_in["wo"],
        "B_x": _B_in["x"],
        "B_w_r": _B_in["w_r"],
        "B_w_gate": _B_in["w_gate"],
        "B_w_up": _B_in["w_up"],
        "B_w_down": _B_in["w_down"],
    }

def reference(A_x, A_k_cache, A_v_cache, A_wq, A_wo, B_x, B_w_r, B_w_gate, B_w_up, B_w_down):
    def _A_ref(x, k_cache, v_cache, wq, wo):
        B, Sq, D = x.shape
        Hq, Dh = 16, 256
        Hkv = k_cache.shape[1]
        rep = Hq // Hkv
        q = (lambda x, *d: x.transpose(*d))((x @ wq).reshape(B, Sq, Hq, Dh), 0, 2, 1, 3)
        k = jnp.repeat(k_cache, rep, axis=1)
        v = jnp.repeat(v_cache, rep, axis=1)
        scores = jnp.einsum("bhqd,bhkd->bhqk", q, k) * (Dh ** -0.5)
        p = _softmax(scores, axis=-1)
        o = jnp.einsum("bhqk,bhkd->bhqd", p, v)
        return (lambda x, *d: x.transpose(*d))(o, 0, 2, 1, 3).reshape(B, Sq, Hq * Dh) @ wo

    def _B_ref(x, w_r, w_gate, w_up, w_down):
        B, S, D = x.shape
        C = 1
        r = x @ w_r
        idx = jnp.argsort(-r, axis=-1)[:, :C]
        idx_e = jnp.repeat(idx.reshape(B, C, 1), D, axis=2)
        x_sel = jnp.take_along_axis(x, idx_e, axis=1)
        g = _silu(x_sel @ w_gate)
        u = x_sel @ w_up
        y = (g * u) @ w_down
        r_sel = _sigmoid(jnp.take_along_axis(r, idx, axis=1))
        y = y * r_sel.reshape(B, C, 1)
        b_off = (jnp.arange(B) * S).reshape(B, 1)
        flat_idx = (idx + b_off).reshape(B * C)
        zero = (x * 0.0).reshape(B * S, D)
        upd = _scatter_add(zero, flat_idx, y.reshape(B * C, D), axis=0)
        return x + upd.reshape(B, S, D)

    x = A_x
    xn = _layernorm(x, axis=-1)
    return x + _A_ref(xn, A_k_cache, A_v_cache, A_wq, A_wo) + _B_ref(xn, B_w_r, B_w_gate, B_w_up, B_w_down)
```

```python
import functools
import jax, jax.numpy as jnp
from jax import lax
from jax.experimental import pallas as pl
from jax.experimental.pallas import tpu as pltpu

bf = jnp.bfloat16
f32 = jnp.float32
D, HQ, HKV, SK, DH, F = 448, 16, 8, 65536, 256, 1792
NT = (((1,), (1,)), ((), ()))
NN = (((1,), (0,)), ((), ()))

def make(G=512, NB=12, t=64, pat=(0, 1), order='issue_first', kv_inter=True, unroll=1):
    GPH = SK // G
    NJ = GPH * HKV
    ns = G // t

    def kernel(x_ref, wr_ref, k_hbm, v_hbm, wq_hbm, wo_hbm, wg_hbm, wu_hbm, wd_hbm, o_ref,
               kbuf, vbuf, wq_v, wo_v, wg_v, wu_v, wd_v, q_s, ksem, vsem, wsem):
        def kcopy(g, slot, i):
            return pltpu.make_async_copy(k_hbm.at[pl.ds(g * G + i * t, t)], kbuf.at[slot, pl.ds(i * t, t)], ksem.at[slot])
        def vcopy(g, slot, i):
            return pltpu.make_async_copy(v_hbm.at[pl.ds(g * G + i * t, t)], vbuf.at[slot, pl.ds(i * t, t)], vsem.at[slot])
        def issue(j, slot, kgran=None):
            gk = jnp.minimum(j + 1, NJ - 1) if kgran is None else kgran
            seq = []
            if kv_inter:
                for i in range(ns): seq += [kcopy(gk, slot, i), vcopy(j, slot, i)]
            else:
                seq = [kcopy(gk, slot, i) for i in range(ns)] + [vcopy(j, slot, i) for i in range(ns)]
            for n, c in enumerate(seq):
                c.start(priority=pat[n % len(pat)])
        def kwait(slot):
            pltpu.make_async_copy(kbuf.at[slot], kbuf.at[slot], ksem.at[slot]).wait()
        def vwait(slot):
            pltpu.make_async_copy(vbuf.at[slot], vbuf.at[slot], vsem.at[slot]).wait()
        wq_cp = [pltpu.make_async_copy(wq_hbm.at[:, pl.ds(h * 512, 512)], wq_v.at[h], wsem.at[h]) for h in range(8)]
        wo_cp = [pltpu.make_async_copy(wo_hbm.at[:, pl.ds(h * 512, 512)], wo_v.at[h], wsem.at[8 + h]) for h in range(8)]
        wg_cp = pltpu.make_async_copy(wg_hbm, wg_v, wsem.at[16])
        wu_cp = pltpu.make_async_copy(wu_hbm, wu_v, wsem.at[17])
        wd_cp = pltpu.make_async_copy(wd_hbm, wd_v, wsem.at[18])

        wq_cp[0].start()
        k0 = pltpu.make_async_copy(k_hbm.at[pl.ds(0, G)], kbuf.at[NB], ksem.at[NB])
        k0.start(priority=1)
        for h in range(1, 8):
            wq_cp[h].start(priority=h % 2)
        wg_cp.start(); wu_cp.start(priority=1); wd_cp.start()
        for h in range(8):
            wo_cp[h].start(priority=(h + 1) % 2)

        x = x_ref[0].astype(f32)
        mu = jnp.mean(x, axis=-1, keepdims=True)
        xc = x - mu
        var = jnp.mean(xc * xc, axis=-1, keepdims=True)
        xn = (xc / jnp.sqrt(var + 1e-5)).astype(bf)
        xn8 = jnp.broadcast_to(xn, (16, D))
        row = lax.broadcasted_iota(jnp.int32, (16, 256), 0)
        for h in range(8):
            wq_cp[h].wait()
            qq = lax.dot_general(xn8, wq_v[h], NN, preferred_element_type=f32)
            qh = jnp.where(row == 0, qq[:, :256], qq[:, 256:])
            q_s[h] = qh.astype(bf)
        wg_cp.wait(); wu_cp.wait(); wd_cp.wait()
        g = lax.dot_general(xn8, wg_v[...], NN, preferred_element_type=f32)
        u = lax.dot_general(xn8, wu_v[...], NN, preferred_element_type=f32)
        g = g.astype(bf).astype(f32); u = u.astype(bf).astype(f32)
        hdn = (g * jax.nn.sigmoid(g) * u).astype(bf)
        y = lax.dot_general(hdn, wd_v[...], NT, preferred_element_type=f32)
        xnf = xn.astype(f32)
        r = jnp.sum(xnf * wr_ref[...].astype(f32).reshape(1, D), axis=-1, keepdims=True)
        base = x + xnf + y[0:1] * jax.nn.sigmoid(r)

        for j in range(NB):
            issue(j, j)

        scale = DH ** -0.5
        def qk(h, slot):
            q = q_s[h]
            s = lax.dot_general(q, kbuf[slot], NT, preferred_element_type=f32)[0:8] * scale
            return s
        def rowmax(s):
            m = s[:, 0:128]
            for i in range(1, G // 128):
                m = jnp.maximum(m, s[:, i * 128:(i + 1) * 128])
            return jnp.max(m, axis=-1, keepdims=True)

        k0.wait()
        s0 = qk(0, NB)
        m0 = rowmax(s0)
        p0 = jnp.exp(s0 - m0)
        a0 = jnp.zeros((8, 1), f32)

        for h in range(8):
            wo_cp[h].wait()

        def step(j, carry):
            p, alpha, m, l, acc = carry
            slot = j % NB
            if order == 'issue_first':
                @pl.when(jnp.logical_and(j >= 1, j - 1 + NB < NJ))
                def _():
                    issue(j - 1 + NB, (j + NB - 1) % NB)
            kwait(slot); vwait(slot)
            hk = jnp.minimum((j + 1) // GPH, 7)
            s = qk(hk, slot)
            first = (j + 1) % GPH == 0
            m_old = jnp.where(first, -jnp.inf, m)
            m_new = jnp.maximum(m_old, rowmax(s))
            alpha_n = jnp.exp(m_old - m_new)
            p_n = jnp.exp(s - m_new)
            pb = jnp.concatenate([p, p], axis=0).astype(bf)
            pv = lax.dot_general(pb, vbuf[slot], NN, preferred_element_type=f32)[0:8]
            ls = p[:, 0:128]
            for i in range(1, G // 128):
                ls = ls + p[:, i * 128:(i + 1) * 128]
            l = alpha * l + ls
            acc = alpha * acc + pv
            if order == 'issue_last':
                @pl.when(j + NB < NJ)
                def _():
                    issue(j + NB, slot)
            return p_n, alpha_n, m_new, l, acc

        row8 = lax.broadcasted_iota(jnp.int32, (8, 256), 0)
        def head(h, carry):
            p, alpha, m, l, acc, out = carry
            p, alpha, m, l, acc = lax.fori_loop(h * GPH, (h + 1) * GPH, step, (p, alpha, m, l, acc), unroll=unroll)
            o = acc / jnp.sum(l, axis=-1, keepdims=True)
            o2 = jnp.concatenate([jnp.where(row8 == 0, o, 0.0), jnp.where(row8 == 1, o, 0.0)], axis=1)
            o2 = jnp.concatenate([o2, o2], axis=0).astype(bf)
            out = out + lax.dot_general(o2, wo_v[h], NT, preferred_element_type=f32)[0:8]
            return p, alpha, m, l, acc, out

        init = (p0, a0, m0, jnp.zeros((8, 128), f32), jnp.zeros((8, 256), f32), jnp.zeros((8, D), f32))
        out = lax.fori_loop(0, 8, head, init)[-1]
        res = base + out[0:1] + out[1:2]
        o_ref[0] = res.astype(bf)

    def fn(A_x, A_k_cache, A_v_cache, A_wq, A_wo, B_x, B_w_r, B_w_gate, B_w_up, B_w_down):
        k = A_k_cache.reshape(HKV * SK, DH); v = A_v_cache.reshape(HKV * SK, DH)
        hbm = pl.BlockSpec(memory_space=pltpu.HBM)
        vm = pl.BlockSpec(memory_space=pltpu.VMEM)
        return pl.pallas_call(
            kernel, out_shape=jax.ShapeDtypeStruct((1, 1, D), bf),
            in_specs=[vm, vm] + [hbm] * 7, out_specs=vm,
            scratch_shapes=[pltpu.VMEM((NB + 1, G, DH), bf), pltpu.VMEM((NB, G, DH), bf),
                            pltpu.VMEM((8, D, 512), bf), pltpu.VMEM((8, D, 512), bf),
                            pltpu.VMEM((D, F), bf), pltpu.VMEM((D, F), bf), pltpu.VMEM((D, F), bf),
                            pltpu.VMEM((8, 16, 256), bf),
                            pltpu.SemaphoreType.DMA((NB + 1,)), pltpu.SemaphoreType.DMA((NB,)), pltpu.SemaphoreType.DMA((19,))],
            compiler_params=pltpu.CompilerParams(vmem_limit_bytes=100 * 1024 * 1024),
        )(A_x, B_w_r, k, v, A_wq, A_wo.T, B_w_gate, B_w_up, B_w_down.T)
    return fn


_fn = make(G=512, NB=12, t=64, pat=(0, 0, 1), order='issue_last')


@jax.jit
def pallas_parallel_sum__gqa_block_cached__moe_arch_mod__decode_kernel(
    A_x, A_k_cache, A_v_cache, A_wq, A_wo, B_x, B_w_r, B_w_gate, B_w_up, B_w_down,
):
    return _fn(A_x, A_k_cache, A_v_cache, A_wq, A_wo, B_x, B_w_r, B_w_gate, B_w_up, B_w_down)
```

```python
import functools
import jax, jax.numpy as jnp
from jax import lax
from jax.experimental import pallas as pl
from jax.experimental.pallas import tpu as pltpu

bf = jnp.bfloat16
f32 = jnp.float32
D, HQ, HKV, SK, DH, F = 448, 16, 8, 65536, 256, 1792
NT = (((1,), (1,)), ((), ()))
NN = (((1,), (0,)), ((), ()))

def make(G=512, NB=16, t=64, pat=(0, 0, 1), kv_inter=True, bc=False, wsplit=1, pre=0, order="last", frac=1, voff=0, vrev=False, blk=1, mi=None, mj=0, vflip=1, base_p=0, prog=None):
    GPH = SK // G // frac
    NJ = GPH * HKV
    ns = G // t

    def kernel(x_hbm, wr_hbm, k_hbm, v_hbm, wq_hbm, wo_hbm, wg_hbm, wu_hbm, wd_hbm, o_ref,
               kbuf, vbuf, wq_v, wo_v, wg_v, wu_v, wd_v, q_s, x_v, wr_v, ksem, vsem, wsem):
        def kcopy(g, slot, i):
            return pltpu.make_async_copy(k_hbm.at[pl.ds(pl.multiple_of(g * G + i * t, t), t)], kbuf.at[slot, pl.ds(pl.multiple_of(i * t, t) if not isinstance(i, int) else i * t, t)], ksem.at[slot])
        def vcopy(g, slot, i):
            return pltpu.make_async_copy(v_hbm.at[pl.ds(pl.multiple_of(g * G + i * t, t), t)], vbuf.at[slot, pl.ds(pl.multiple_of(i * t, t) if not isinstance(i, int) else i * t, t)], vsem.at[slot])
        def par(x):
            x = x & mj
            r = 0
            for b in range(12):
                if (mj >> b) & 1: r = r ^ (x >> b)
            return r & 1
        def popc(i): return bin(i).count('1') & 1
        def issue(j, slot):
            if prog is not None:
                pos = {'k': 0, 'v': 0}
                n = 0
                while pos['k'] < G or pos['v'] < G:
                    w, r, p = prog[n % len(prog)]; n += 1
                    r = min(r, G - pos[w])
                    if r <= 0: continue
                    if w == 'k':
                        c = pltpu.make_async_copy(k_hbm.at[pl.ds((j + 1) * G + pos[w], r)], kbuf.at[slot, pl.ds(pos[w], r)], ksem.at[slot])
                    else:
                        c = pltpu.make_async_copy(v_hbm.at[pl.ds(j * G + pos[w], r)], vbuf.at[slot, pl.ds(pos[w], r)], vsem.at[slot])
                    c.start(priority=p)
                    pos[w] += r
                return
            if mi is not None:
                bit = mi & (-mi)
                fk = par(j + 1) * bit; fv = par(j) * bit
                for i0 in range(0, ns, blk):
                    for i in range(i0, i0 + blk):
                        kcopy(j + 1, slot, i ^ fk).start(priority=popc(i & mi) ^ base_p)
                    for i in range(i0, i0 + blk):
                        vcopy(j, slot, i ^ fv).start(priority=popc(i & mi) ^ vflip ^ base_p)
                return
            seq = []
            if kv_inter:
                for i0 in range(0, ns, blk):
                    seq += [kcopy(j + 1, slot, i) for i in range(i0, i0 + blk)]
                    seq += [vcopy(j, slot, ((ns - 1 - i) if vrev else (i + voff) % ns)) for i in range(i0, i0 + blk)]
            else:
                seq = [kcopy(j + 1, slot, i) for i in range(ns)] + [vcopy(j, slot, i) for i in range(ns)]
            for n, c in enumerate(seq):
                c.start(priority=pat[n % len(pat)])
        def issue_v(j, slot):
            for i in range(ns):
                vcopy(j, slot, i).start(priority=pat[i % len(pat)])
        def kwait(slot):
            pltpu.make_async_copy(kbuf.at[slot], kbuf.at[slot], ksem.at[slot]).wait()
        def vwait(slot):
            pltpu.make_async_copy(vbuf.at[slot], vbuf.at[slot], vsem.at[slot]).wait()

        def split_copies(src, dst, sem, nrows):
            r = 448 // wsplit
            return [pltpu.make_async_copy(src.at[pl.ds(i * r, r)], dst.at[pl.ds(i * r, r)], sem) for i in range(wsplit)]
        cnt = [0]
        def start_all(cs):
            for c in cs:
                c.start(priority=cnt[0] % 2); cnt[0] += 1
        def wait_all(cs):
            for c in cs: c.wait()
        wq_cp = [split_copies(wq_hbm.at[:, pl.ds(h * 512, 512)], wq_v.at[h], wsem.at[h], D) for h in range(8)]
        wo_cp = [split_copies(wo_hbm.at[:, pl.ds(h * 512, 512)], wo_v.at[h], wsem.at[8 + h], D) for h in range(8)]
        wg_cp = split_copies(wg_hbm, wg_v, wsem.at[16], D)
        wu_cp = split_copies(wu_hbm, wu_v, wsem.at[17], D)
        wd_cp = split_copies(wd_hbm, wd_v, wsem.at[18], D)
        x_cp = pltpu.make_async_copy(x_hbm, x_v, wsem.at[19])
        wr_cp = pltpu.make_async_copy(wr_hbm, wr_v, wsem.at[20])

        x_cp.start()
        start_all(wq_cp[0])
        k0 = pltpu.make_async_copy(k_hbm.at[pl.ds(0, G)], kbuf.at[NB], ksem.at[NB])
        k0.start(priority=1)
        wr_cp.start()
        for h in range(1, 8):
            start_all(wq_cp[h])
        start_all(wg_cp); start_all(wu_cp); start_all(wd_cp)
        for h in range(8):
            start_all(wo_cp[h])
        for j in range(pre):
            issue(j, j)

        x_cp.wait()
        x = x_v[0].astype(f32)
        mu = jnp.mean(x, axis=-1, keepdims=True)
        xc = x - mu
        var = jnp.mean(xc * xc, axis=-1, keepdims=True)
        xn = (xc / jnp.sqrt(var + 1e-5)).astype(bf)
        xn8 = jnp.broadcast_to(xn, (16, D))
        row = lax.broadcasted_iota(jnp.int32, (16, 256), 0)
        for h in range(8):
            wait_all(wq_cp[h])
            qq = lax.dot_general(xn8, wq_v[h], NN, preferred_element_type=f32)
            qh = jnp.where(row == 0, qq[:, :256], qq[:, 256:])
            q_s[h] = qh.astype(bf)
        wait_all(wg_cp); wait_all(wu_cp)
        g = lax.dot_general(xn8, wg_v[...], NN, preferred_element_type=f32)
        u = lax.dot_general(xn8, wu_v[...], NN, preferred_element_type=f32)
        g = g.astype(bf).astype(f32); u = u.astype(bf).astype(f32)
        hdn = (g * jax.nn.sigmoid(g) * u).astype(bf)
        wait_all(wd_cp)
        y = lax.dot_general(hdn, wd_v[...], NT, preferred_element_type=f32)
        xnf = xn.astype(f32)
        wr_cp.wait()
        r = jnp.sum(xnf * wr_v[...].astype(f32).reshape(1, D), axis=-1, keepdims=True)
        base = x + xnf + y[0:1] * jax.nn.sigmoid(r)

        for j in range(pre, NB):
            issue(j, j)

        scale = DH ** -0.5
        def qk(h, slot):
            q = q_s[h]
            s = lax.dot_general(q, kbuf[slot], NT, preferred_element_type=f32)[0:8] * scale
            return s
        def rowmax(s):
            m = s[:, 0:128]
            for i in range(1, G // 128):
                m = jnp.maximum(m, s[:, i * 128:(i + 1) * 128])
            return jnp.max(m, axis=-1, keepdims=True)

        k0.wait()
        s0 = qk(0, NB)
        m0 = rowmax(s0)
        p0 = jnp.exp(s0 - m0)
        a0 = jnp.zeros((8, 1), f32)

        for h in range(8):
            wait_all(wo_cp[h])

        def refill(jn, slot):
            @pl.when(jn < NJ - 1)
            def _():
                issue(jn, slot)
            @pl.when(jn == NJ - 1)
            def _():
                issue_v(jn, slot)

        def step(j, carry):
            p, alpha, m, l, acc = carry
            slot = j % NB
            if order == 'first':
                @pl.when(j >= 1)
                def _():
                    refill(j - 1 + NB, (j + NB - 1) % NB)
            @pl.when(j < NJ - 1)
            def _():
                kwait(slot)
            vwait(slot)
            hk = jnp.minimum((j + 1) // GPH, 7)
            s = qk(hk, slot)
            first = (j + 1) % GPH == 0
            m_old = jnp.where(first, -jnp.inf, m)
            m_new = jnp.maximum(m_old, rowmax(s))
            alpha_n = jnp.exp(m_old - m_new)
            p_n = jnp.exp(s - m_new)
            pb = jnp.concatenate([p, p], axis=0).astype(bf)
            pv = lax.dot_general(pb, vbuf[slot], NN, preferred_element_type=f32)[0:8]
            ls = p[:, 0:128]
            for i in range(1, G // 128):
                ls = ls + p[:, i * 128:(i + 1) * 128]
            l = alpha * l + ls
            acc = alpha * acc + pv
            if order == 'last':
                refill(j + NB, slot)
            return p_n, alpha_n, m_new, l, acc

        row8 = lax.broadcasted_iota(jnp.int32, (8, 256), 0)
        def head(h, carry):
            p, alpha, m, l, acc, out = carry
            p, alpha, m, l, acc = lax.fori_loop(h * GPH, (h + 1) * GPH, step, (p, alpha, m, l, acc))
            o = acc / jnp.sum(l, axis=-1, keepdims=True)
            o2 = jnp.concatenate([jnp.where(row8 == 0, o, 0.0), jnp.where(row8 == 1, o, 0.0)], axis=1)
            o2 = jnp.concatenate([o2, o2], axis=0).astype(bf)
            out = out + lax.dot_general(o2, wo_v[h], NT, preferred_element_type=f32)[0:8]
            return p, alpha, m, l, acc, out

        init = (p0, a0, m0, jnp.zeros((8, 128), f32), jnp.zeros((8, 256), f32), jnp.zeros((8, D), f32))
        out = lax.fori_loop(0, 8, head, init)[-1]
        res = base + out[0:1] + out[1:2]
        o_ref[0] = res.astype(bf)

    def fn(A_x, A_k_cache, A_v_cache, A_wq, A_wo, B_x, B_w_r, B_w_gate, B_w_up, B_w_down):
        k = A_k_cache.reshape(HKV * SK, DH); v = A_v_cache.reshape(HKV * SK, DH)
        hbm = pl.BlockSpec(memory_space=pltpu.HBM)
        vm = pl.BlockSpec(memory_space=pltpu.VMEM)
        return pl.pallas_call(
            kernel, out_shape=jax.ShapeDtypeStruct((1, 1, D), bf),
            in_specs=[hbm] * 9, out_specs=vm,
            scratch_shapes=[pltpu.VMEM((NB + 1, G, DH), bf), pltpu.VMEM((NB, G, DH), bf),
                            pltpu.VMEM((8, D, 512), bf), pltpu.VMEM((8, D, 512), bf),
                            pltpu.VMEM((D, F), bf), pltpu.VMEM((D, F), bf), pltpu.VMEM((D, F), bf),
                            pltpu.VMEM((8, 16, 256), bf), pltpu.VMEM((1, 1, D), bf), pltpu.VMEM((D,), bf),
                            pltpu.SemaphoreType.DMA((NB + 1,)), pltpu.SemaphoreType.DMA((NB,)), pltpu.SemaphoreType.DMA((21,))],
            compiler_params=pltpu.CompilerParams(vmem_limit_bytes=100 * 1024 * 1024, disable_bounds_checks=not bc),
        )(A_x, B_w_r, k, v, A_wq, A_wo.T, B_w_gate, B_w_up, B_w_down.T)
    return fn


_fn = make(G=1024, NB=8, t=64, pat=(0, 1, 1, 0, 1, 0, 0, 1), wsplit=7)


@jax.jit
def pallas_parallel_sum__gqa_block_cached__moe_arch_mod__decode_kernel(
    A_x, A_k_cache, A_v_cache, A_wq, A_wo, B_x, B_w_r, B_w_gate, B_w_up, B_w_down,
):
    return _fn(A_x, A_k_cache, A_v_cache, A_wq, A_wo, B_x, B_w_r, B_w_gate, B_w_up, B_w_down)
```

```python
import jax
import jax.numpy as jnp
from jax import lax
from jax.experimental import pallas as pl
from jax.experimental.pallas import tpu as pltpu

bf = jnp.bfloat16
f32 = jnp.float32
D, HKV, SK, DH, F = 448, 8, 65536, 256, 1792
NT = (((1,), (1,)), ((), ()))
NN = (((1,), (0,)), ((), ()))
G, NB = 1024, 5
GPH = SK // G
NJ = GPH * HKV
WSPLIT = 14


def _pieces(shift, split, flip, blk=128):
    out, n = [], -1
    while shift + n * blk < G:
        pos = shift + n * blk
        for r in split:
            a, e = max(pos, 0), min(pos + r, G)
            if e > a:
                out.append((a, e - a, (n & 1) ^ flip))
            pos += r
        n += 1
    return out


KP = _pieces(64, (64, 64), 0)
VP = _pieces(32, (112, 16), 1)


def _kernel(x_hbm, wr_hbm, k_hbm, v_hbm, wq_hbm, wo_hbm, wg_hbm, wu_hbm, wd_hbm, o_ref,
            kbuf, vbuf, wq_v, wo_v, wg_v, wu_v, wd_v, q_s, x_v, wr_v, ksem, vsem, wsem):
    def start_piece(src, buf, sem, g, slot, piece):
        a, r, p = piece
        pltpu.make_async_copy(src.at[pl.ds(g * G + a, r)], buf.at[slot, pl.ds(a, r)], sem.at[slot]).start(priority=p)

    def issue(j, slot, with_k=True):
        for i in range(max(len(KP), len(VP))):
            if with_k and i < len(KP):
                start_piece(k_hbm, kbuf, ksem, j + 1, slot, KP[i])
            if i < len(VP):
                start_piece(v_hbm, vbuf, vsem, j, slot, VP[i])

    def wait_slot(buf, sem, slot):
        pltpu.make_async_copy(buf.at[slot], buf.at[slot], sem.at[slot]).wait()

    def split_copies(src, dst, sem):
        r = D // WSPLIT
        return [pltpu.make_async_copy(src.at[pl.ds(i * r, r)], dst.at[pl.ds(i * r, r)], sem) for i in range(WSPLIT)]

    def start_all(cs):
        for i, c in enumerate(cs):
            c.start(priority=i % 2)

    def wait_all(cs):
        for c in cs:
            c.wait()

    wq_cp = [split_copies(wq_hbm.at[:, pl.ds(h * 512, 512)], wq_v.at[h], wsem.at[h]) for h in range(HKV)]
    wo_cp = [split_copies(wo_hbm.at[:, pl.ds(h * 512, 512)], wo_v.at[h], wsem.at[8 + h]) for h in range(HKV)]
    wg_cp = split_copies(wg_hbm, wg_v, wsem.at[16])
    wu_cp = split_copies(wu_hbm, wu_v, wsem.at[17])
    wd_cp = split_copies(wd_hbm, wd_v, wsem.at[18])
    x_cp = pltpu.make_async_copy(x_hbm, x_v, wsem.at[19])
    wr_cp = pltpu.make_async_copy(wr_hbm, wr_v, wsem.at[20])
    k0_cp = pltpu.make_async_copy(k_hbm.at[pl.ds(0, G)], kbuf.at[NB], ksem.at[NB])

    x_cp.start()
    start_all(wq_cp[0])
    k0_cp.start(priority=1)
    wr_cp.start()
    for h in range(1, HKV):
        start_all(wq_cp[h])
    start_all(wg_cp)
    start_all(wu_cp)
    start_all(wd_cp)
    for h in range(HKV):
        start_all(wo_cp[h])

    x_cp.wait()
    x = x_v[0].astype(f32)
    xc = x - jnp.mean(x, axis=-1, keepdims=True)
    var = jnp.mean(xc * xc, axis=-1, keepdims=True)
    xn = (xc / jnp.sqrt(var + 1e-5)).astype(bf)
    xn16 = jnp.broadcast_to(xn, (16, D))

    row = lax.broadcasted_iota(jnp.int32, (16, DH), 0)
    for h in range(HKV):
        wait_all(wq_cp[h])
        qq = lax.dot_general(xn16, wq_v[h], NN, preferred_element_type=f32)
        q_s[h] = jnp.where(row == 0, qq[:, :DH], qq[:, DH:]).astype(bf)

    wait_all(wg_cp)
    wait_all(wu_cp)
    g = lax.dot_general(xn16, wg_v[...], NN, preferred_element_type=f32).astype(bf).astype(f32)
    u = lax.dot_general(xn16, wu_v[...], NN, preferred_element_type=f32).astype(bf).astype(f32)
    hdn = (g * jax.nn.sigmoid(g) * u).astype(bf)
    wait_all(wd_cp)
    y = lax.dot_general(hdn, wd_v[...], NT, preferred_element_type=f32)
    xnf = xn.astype(f32)
    wr_cp.wait()
    r = jnp.sum(xnf * wr_v[...].astype(f32).reshape(1, D), axis=-1, keepdims=True)
    base = x + xnf + y[0:1] * jax.nn.sigmoid(r)

    for j in range(NB):
        issue(j, j)

    def qk(h, slot):
        return lax.dot_general(q_s[h], kbuf[slot], NT, preferred_element_type=f32)[0:8] * (DH ** -0.5)

    def rowmax(s):
        m = s[:, 0:128]
        for i in range(1, G // 128):
            m = jnp.maximum(m, s[:, i * 128:(i + 1) * 128])
        return jnp.max(m, axis=-1, keepdims=True)

    k0_cp.wait()
    s0 = qk(0, NB)
    m0 = rowmax(s0)
    p0 = jnp.exp(s0 - m0)
    for h in range(HKV):
        wait_all(wo_cp[h])

    def step(j, carry):
        p, alpha, m, l, acc = carry
        slot = j % NB

        @pl.when(j < NJ - 1)
        def _():
            wait_slot(kbuf, ksem, slot)
        wait_slot(vbuf, vsem, slot)

        s = qk(jnp.minimum((j + 1) // GPH, HKV - 1), slot)
        m_old = jnp.where((j + 1) % GPH == 0, -jnp.inf, m)
        m_new = jnp.maximum(m_old, rowmax(s))
        alpha_n = jnp.exp(m_old - m_new)
        p_n = jnp.exp(s - m_new)

        pb = jnp.concatenate([p, p], axis=0).astype(bf)
        pv = lax.dot_general(pb, vbuf[slot], NN, preferred_element_type=f32)[0:8]
        ls = p[:, 0:128]
        for i in range(1, G // 128):
            ls = ls + p[:, i * 128:(i + 1) * 128]
        l = alpha * l + ls
        acc = alpha * acc + pv

        @pl.when(j + NB < NJ - 1)
        def _():
            issue(j + NB, slot)

        @pl.when(j + NB == NJ - 1)
        def _():
            issue(j + NB, slot, with_k=False)
        return p_n, alpha_n, m_new, l, acc

    row8 = lax.broadcasted_iota(jnp.int32, (8, DH), 0)

    def head(h, carry):
        p, alpha, m, l, acc = lax.fori_loop(h * GPH, (h + 1) * GPH, step, carry[:5])
        o = acc / jnp.sum(l, axis=-1, keepdims=True)
        o2 = jnp.concatenate([jnp.where(row8 == 0, o, 0.0), jnp.where(row8 == 1, o, 0.0)], axis=1)
        o2 = jnp.concatenate([o2, o2], axis=0).astype(bf)
        out = carry[5] + lax.dot_general(o2, wo_v[h], NT, preferred_element_type=f32)[0:8]
        return p, alpha, m, l, acc, out

    init = (p0, jnp.zeros((8, 1), f32), m0, jnp.zeros((8, 128), f32), jnp.zeros((8, DH), f32), jnp.zeros((8, D), f32))
    out = lax.fori_loop(0, HKV, head, init)[-1]
    o_ref[0] = (base + out[0:1] + out[1:2]).astype(bf)


@jax.jit
def pallas_parallel_sum__gqa_block_cached__moe_arch_mod__decode_kernel(
    A_x, A_k_cache, A_v_cache, A_wq, A_wo, B_x, B_w_r, B_w_gate, B_w_up, B_w_down,
):
    del B_x
    return pl.pallas_call(
        _kernel,
        out_shape=jax.ShapeDtypeStruct((1, 1, D), bf),
        in_specs=[pl.BlockSpec(memory_space=pltpu.HBM)] * 9,
        out_specs=pl.BlockSpec(memory_space=pltpu.VMEM),
        scratch_shapes=[
            pltpu.VMEM((NB + 1, G, DH), bf), pltpu.VMEM((NB, G, DH), bf),
            pltpu.VMEM((HKV, D, 512), bf), pltpu.VMEM((HKV, D, 512), bf),
            pltpu.VMEM((D, F), bf), pltpu.VMEM((D, F), bf), pltpu.VMEM((D, F), bf),
            pltpu.VMEM((HKV, 16, DH), bf), pltpu.VMEM((1, 1, D), bf), pltpu.VMEM((D,), bf),
            pltpu.SemaphoreType.DMA((NB + 1,)), pltpu.SemaphoreType.DMA((NB,)), pltpu.SemaphoreType.DMA((21,)),
        ],
        compiler_params=pltpu.CompilerParams(vmem_limit_bytes=100 * 1024 * 1024, disable_bounds_checks=True),
    )(A_x, B_w_r, A_k_cache.reshape(HKV * SK, DH), A_v_cache.reshape(HKV * SK, DH),
      A_wq, A_wo.T, B_w_gate, B_w_up, B_w_down.T)
```
